```python
import jax
import jax.numpy as jnp

def _softmax(x, axis=-1):
    return jax.nn.softmax(x, axis=axis)

def _gelu(x):
    return jax.nn.gelu(x, approximate=True)

def _silu(x):
    return jax.nn.silu(x)

def _sigmoid(x):
    return jax.nn.sigmoid(x)

def _layernorm(x, axis=-1, eps=1e-05):
    m = jnp.mean(x, axis=axis, keepdims=True)
    v = jnp.var(x, axis=axis, keepdims=True)
    return (x - m) / jnp.sqrt(v + eps)

def _scatter_add(tgt, idx, src, axis=0):
    return tgt.at[idx].add(src)

def _segment_sum(src, seg, n):
    return jax.ops.segment_sum(src, seg, n)

class _Rng:

    def __init__(self, key):
        self._k = key

    def _next(self):
        self._k, sub = jax.random.split(self._k)
        return sub

    def normal(self, shape):
        return jax.random.normal(self._next(), shape, dtype=jnp.bfloat16)

    def randint(self, lo, hi, shape):
        return jax.random.randint(self._next(), shape, lo, hi, dtype=jnp.int32)

    def uniform(self, shape, lo=0.0, hi=1.0):
        return jax.random.uniform(self._next(), shape, jnp.bfloat16, lo, hi)

    def permutation(self, n):
        return jax.random.permutation(self._next(), n)
kernel_name = 'recurrent_scan__memory_aug_recurrent_mem_tr__glu_gated_glu__prompt'

def setup_inputs():
    _rng = _Rng(jax.random.key(int.from_bytes(__import__("os").urandom(4), "little")))
    _w = lambda a: (lambda t: t.astype(jnp.bfloat16) if jnp.issubdtype(t.dtype, jnp.floating) else t)(jnp.asarray(a))

    def _A_setup():
        B, S, Dm = (1, 2048, 1024)
        H, Dh = (32, 128)
        M, seg = (8, 32)
        seg = min(seg, S)
        S = S // seg * seg
        return {'x': _w((lambda *s: _rng.normal(s) * 0.05)(B, S, Dm)), 'mem0': _w((lambda *s: _rng.normal(s) * 0.05)(B, M, Dm)), 'Wq': _w((lambda *s: _rng.normal(s) * 0.05)(Dm, H, Dh) * Dm ** (-0.5)), 'Wk': _w((lambda *s: _rng.normal(s) * 0.05)(Dm, H, Dh) * Dm ** (-0.5)), 'Wv': _w((lambda *s: _rng.normal(s) * 0.05)(Dm, H, Dh) * Dm ** (-0.5)), 'Wo': _w((lambda *s: _rng.normal(s) * 0.05)(H, Dh, Dm) * (H * Dh) ** (-0.5)), 'seg_len': seg}
    _A_in = _A_setup()

    def _B_setup():
        B, S, D, F = (1, 2048, 1024, 3584)
        return {'x': _w((lambda *s: _rng.normal(s) * 0.05)(B, S, D)), 'w_gate': _w((lambda *s: _rng.normal(s) * 0.05)(D, F)), 'w_up': _w((lambda *s: _rng.normal(s) * 0.05)(D, F)), 'w_down': _w((lambda *s: _rng.normal(s) * 0.05)(F, D))}
    _B_in = _B_setup()
    return {'A_x': _A_in['x'], 'A_mem0': _A_in['mem0'], 'A_Wq': _A_in['Wq'], 'A_Wk': _A_in['Wk'], 'A_Wv': _A_in['Wv'], 'A_Wo': _A_in['Wo'], 'A_seg_len': _A_in['seg_len'], 'B_x': _B_in['x'], 'B_w_gate': _B_in['w_gate'], 'B_w_up': _B_in['w_up'], 'B_w_down': _B_in['w_down']}

def reference(A_x, A_mem0, A_Wq, A_Wk, A_Wv, A_Wo, A_seg_len, B_x, B_w_gate, B_w_up, B_w_down):

    def _A_ref(x, mem0, Wq, Wk, Wv, Wo, seg_len):
        B, S, Dm = x.shape
        H, Dh = (Wq.shape[1], Wq.shape[2])
        M = mem0.shape[1]
        scale = Dh ** (-0.5)
        n_seg = S // seg_len
        L = M + seg_len
        idx = jnp.arange(L)
        mask = (idx[:, None] < M) | (idx[:, None] >= idx[None, :])
        mem = mem0
        outs = []
        for s in range(n_seg):
            xs = x[:, s * seg_len:(s + 1) * seg_len, :].copy()
            h = jnp.concatenate([mem, xs], axis=1)
            q = jnp.einsum('btd,dhe->bhte', h, Wq)
            k = jnp.einsum('btd,dhe->bhte', h, Wk)
            v = jnp.einsum('btd,dhe->bhte', h, Wv)
            scores = jnp.einsum('bhqe,bhke->bhqk', q, k) * scale
            scores = jnp.where(mask[None, None], scores, -1000000000.0)
            p = _softmax(scores, axis=-1)
            o = jnp.einsum('bhqk,bhke->bhqe', p, v)
            o = jnp.einsum('bhte,hed->btd', o, Wo)
            mem = o[:, :M, :].copy()
            outs.append(o[:, M:, :])
        return jnp.concatenate(outs, axis=1)

    def _B_ref(x, w_gate, w_up, w_down):
        g = jnp.einsum('bsd,df->bsf', x, w_gate)
        u = jnp.einsum('bsd,df->bsf', x, w_up)
        h = _sigmoid(g) * u
        return jnp.einsum('bsf,fd->bsd', h, w_down)
    x = A_x
    xn = _layernorm(x, axis=-1)
    s = _A_ref(xn, A_mem0, A_Wq, A_Wk, A_Wv, A_Wo, A_seg_len)
    g = _silu(_B_ref(xn, B_w_gate, B_w_up, B_w_down))
    return x + s * g
```

```python
import functools
import numpy as np
import jax
import jax.numpy as jnp
from jax import lax
from jax.experimental import pallas as pl
from jax.experimental.pallas import tpu as pltpu

_F32 = jnp.float32
_BF16 = jnp.bfloat16
_U32 = jnp.uint32


def _make_kernel(S, D, H, Dh, M, seg, F, FC, RB):
    n_pair = S // (2 * seg)
    PR = 2 * seg
    RA = seg - M
    n_fc = F // FC
    n_rb = S // RB
    scale = float(Dh) ** -0.5
    L = M + seg

    def kernel(x_hbm, mem0_ref, wq_hbm, wk_hbm, wv_hbm, wo_hbm, wg_hbm, wu_hbm, wd_hbm,
               out_ref,
               x_v, xn_v, acc_v, wg_b, wu_b, wd_b,
               st_q, st_k, st_v, st_o, wq_p, wk_p, wv_p, wo_p,
               qkv_buf, o_buf, sems):
        def mlp_copies(c, slot):
            c0 = pl.multiple_of(c * FC, FC)
            return (
                pltpu.make_async_copy(wg_hbm.at[:, pl.ds(c0, FC)], wg_b.at[slot], sems.at[0 + slot]),
                pltpu.make_async_copy(wu_hbm.at[:, pl.ds(c0, FC)], wu_b.at[slot], sems.at[2 + slot]),
                pltpu.make_async_copy(wd_hbm.at[pl.ds(c0, FC), :], wd_b.at[slot], sems.at[4 + slot]),
            )
        cp_x = pltpu.make_async_copy(x_hbm, x_v, sems.at[6])
        cp_x.start()
        for cp in mlp_copies(0, 0):
            cp.start()
        cp_a = (
            pltpu.make_async_copy(wq_hbm, st_q, sems.at[7]),
            pltpu.make_async_copy(wk_hbm, st_k, sems.at[8]),
            pltpu.make_async_copy(wv_hbm, st_v, sems.at[9]),
            pltpu.make_async_copy(wo_hbm, st_o, sems.at[10]),
        )
        for cp in cp_a:
            cp.start()

        cp_x.wait()

        def ln_body(r, _):
            r0 = pl.multiple_of(r * 256, 256)
            xv = x_v[pl.ds(r0, 256), :].astype(_F32)
            mu = jnp.mean(xv, axis=-1, keepdims=True)
            xc = xv - mu
            var = jnp.mean(xc * xc, axis=-1, keepdims=True)
            xn_v[pl.ds(r0, 256), :] = (xc * lax.rsqrt(var + 1e-5)).astype(_BF16)
            acc_v[pl.ds(r0, 256), :] = jnp.zeros((256, D), _F32)
            return 0
        lax.fori_loop(0, S // 256, ln_body, 0)

        def mlp_chunk(c, _):
            slot = lax.rem(c, 2)

            @pl.when(c + 1 < n_fc)
            def _():
                for cp in mlp_copies(c + 1, 1 - slot):
                    cp.start()
            for cp in mlp_copies(c, slot):
                cp.wait()

            def rb_body(r, _):
                r0 = pl.multiple_of(r * RB, RB)
                xb = xn_v[pl.ds(r0, RB), :]
                g = jnp.dot(xb, wg_b[slot], preferred_element_type=_F32)
                u = jnp.dot(xb, wu_b[slot], preferred_element_type=_F32)
                h = (jax.nn.sigmoid(g) * u).astype(_BF16)
                acc_v[pl.ds(r0, RB), :] += jnp.dot(h, wd_b[slot], preferred_element_type=_F32)
                return 0
            lax.fori_loop(0, n_rb, rb_body, 0)
            return 0
        lax.fori_loop(0, n_fc, mlp_chunk, 0)

        for cp in cp_a:
            cp.wait()

        def conv3(stage, dst):
            def body(i, _):
                d0 = pl.multiple_of(i * 16, 16)
                v = stage[pl.ds(d0, 16), :, :]
                u = pltpu.bitcast(v, _U32).reshape(8, 2, H // 2, Dh)
                ev = jnp.swapaxes(u[:, 0], 0, 1)
                od = jnp.swapaxes(u[:, 1], 0, 1)
                lo = (ev & jnp.uint32(0xFFFF)) | (od << 16)
                hi = (ev >> 16) | (od & jnp.uint32(0xFFFF0000))
                r0 = pl.multiple_of(i * 8, 8)
                for hp in range(H // 2):
                    dst[2 * hp, pl.ds(r0, 8), :] = lo[hp]
                    dst[2 * hp + 1, pl.ds(r0, 8), :] = hi[hp]
                return 0
            lax.fori_loop(0, D // 16, body, 0)
        conv3(st_q, wq_p)
        conv3(st_k, wk_p)
        conv3(st_v, wv_p)

        def convo(h, _):
            wo_p[h] = pltpu.bitcast(st_o[h], _U32)
            return 0
        lax.fori_loop(0, H, convo, 0)

        def W(ref, h):
            return pltpu.bitcast(ref[h], _BF16)

        x0 = xn_v[pl.ds(0, PR), :]
        for h in range(H):
            for t, wp in enumerate((wq_p, wk_p, wv_p)):
                qkv_buf[0, t * H + h] = jnp.dot(x0, W(wp, h), preferred_element_type=_F32)
        o_buf[1] = jnp.zeros((H, PR, Dh), _F32)

        row = lax.broadcasted_iota(jnp.int32, (L, L), 0)
        col = lax.broadcasted_iota(jnp.int32, (L, L), 1)
        mask = (row < M) | (row >= col)

        def step(mem, cur, nxt, xrow0, seg_off, off, nrows):
            xr = xn_v[pl.ds(xrow0, nrows), :].astype(_F32)
            lhs = jnp.concatenate([mem, xr], axis=0).astype(_BF16)
            acc = None
            for h in range(H):
                qa = jnp.dot(lhs, W(wq_p, h), preferred_element_type=_F32)
                ka = jnp.dot(lhs, W(wk_p, h), preferred_element_type=_F32)
                va = jnp.dot(lhs, W(wv_p, h), preferred_element_type=_F32)
                qkv_buf[nxt, h, pl.ds(off, nrows), :] = qa[M:]
                qkv_buf[nxt, H + h, pl.ds(off, nrows), :] = ka[M:]
                qkv_buf[nxt, 2 * H + h, pl.ds(off, nrows), :] = va[M:]
                q = jnp.concatenate([qa[:M], qkv_buf[cur, h, pl.ds(seg_off, seg), :]], 0).astype(_BF16)
                k = jnp.concatenate([ka[:M], qkv_buf[cur, H + h, pl.ds(seg_off, seg), :]], 0).astype(_BF16)
                v = jnp.concatenate([va[:M], qkv_buf[cur, 2 * H + h, pl.ds(seg_off, seg), :]], 0).astype(_BF16)
                s = lax.dot_general(q, k, (((1,), (1,)), ((), ())), preferred_element_type=_F32) * scale
                s = jnp.where(mask, s, -1e9)
                m = jnp.max(s, axis=-1, keepdims=True)
                e = jnp.exp(s - m)
                p = e / jnp.sum(e, axis=-1, keepdims=True)
                o = jnp.dot(p.astype(_BF16), v, preferred_element_type=_F32)
                o_buf[cur, h, pl.ds(seg_off, seg), :] = o[M:]
                lo = jnp.concatenate([o[:M], o_buf[nxt, h, pl.ds(off, nrows), :]], 0).astype(_BF16)
                part = jnp.dot(lo, W(wo_p, h), preferred_element_type=_F32)
                acc = part if acc is None else acc + part
            new_mem = acc[:M].astype(_BF16).astype(_F32)
            return new_mem, acc[M:]

        def finish(r0, nrows, s_rows):
            xv = x_v[pl.ds(r0, nrows), :].astype(_F32)
            gate = jax.nn.silu(acc_v[pl.ds(r0, nrows), :])
            out_ref[pl.ds(r0, nrows), :] = (xv + s_rows * gate).astype(out_ref.dtype)

        def pair_body(j, mem):
            cur = lax.rem(j, 2)
            nxt = 1 - cur
            jn = jnp.minimum(j + 1, n_pair - 1)
            xrow = pl.multiple_of(jn * PR, PR)
            mem, sA = step(mem, cur, nxt, xrow, 0, 0, RA)
            mem, sB = step(mem, cur, nxt, xrow + RA, seg, RA, PR - RA)

            @pl.when(j > 0)
            def _():
                r0 = pl.multiple_of((j - 1) * PR, PR)
                finish(r0, PR, jnp.concatenate([sA, sB], axis=0))
            return mem

        mem = lax.fori_loop(0, n_pair, pair_body, mem0_ref[...].astype(_F32))

        last = (n_pair - 1) % 2
        acc = None
        for h in range(H):
            part = jnp.dot(o_buf[last, h].astype(_BF16), W(wo_p, h), preferred_element_type=_F32)
            acc = part if acc is None else acc + part
        finish(S - PR, PR, acc)

    return kernel


@functools.partial(jax.jit, static_argnames=("A_seg_len",))
def pallas_recurrent_scan__memory_aug_recurrent_mem_tr__glu_gated_glu__prompt_kernel(
        A_x, A_mem0, A_Wq, A_Wk, A_Wv, A_Wo, A_seg_len, B_x, B_w_gate, B_w_up, B_w_down):
    B, S, D = A_x.shape
    assert B == 1
    H, Dh = A_Wq.shape[1], A_Wq.shape[2]
    M = A_mem0.shape[1]
    seg = int(A_seg_len)
    F = B_w_gate.shape[1]
    FC, RB = 512, 512
    PR = 2 * seg
    kernel = _make_kernel(S, D, H, Dh, M, seg, F, FC, RB)
    anyspec = pl.BlockSpec(memory_space=pl.ANY)
    out = pl.pallas_call(
        kernel,
        out_shape=jax.ShapeDtypeStruct((S, D), A_x.dtype),
        in_specs=[anyspec, pl.BlockSpec(memory_space=pltpu.VMEM)] + [anyspec] * 7,
        out_specs=pl.BlockSpec(memory_space=pltpu.VMEM),
        scratch_shapes=[
            pltpu.VMEM((S, D), _BF16), pltpu.VMEM((S, D), _BF16), pltpu.VMEM((S, D), _F32),
            pltpu.VMEM((2, D, FC), _BF16), pltpu.VMEM((2, D, FC), _BF16), pltpu.VMEM((2, FC, D), _BF16),
            pltpu.VMEM((D, H, Dh), _BF16), pltpu.VMEM((D, H, Dh), _BF16), pltpu.VMEM((D, H, Dh), _BF16),
            pltpu.VMEM((H, Dh, D), _BF16),
            pltpu.VMEM((H, D // 2, Dh), _U32), pltpu.VMEM((H, D // 2, Dh), _U32),
            pltpu.VMEM((H, D // 2, Dh), _U32), pltpu.VMEM((H, Dh // 2, D), _U32),
            pltpu.VMEM((2, 3 * H, PR, Dh), _F32), pltpu.VMEM((2, H, PR, Dh), _F32),
            pltpu.SemaphoreType.DMA((11,)),
        ],
        compiler_params=pltpu.CompilerParams(vmem_limit_bytes=120 * 1024 * 1024),
    )(A_x.reshape(S, D), A_mem0.reshape(M, D), A_Wq, A_Wk, A_Wv, A_Wo, B_w_gate, B_w_up, B_w_down)
    return out.reshape(B, S, D)
```

```python
import functools
import numpy as np
import jax
import jax.numpy as jnp
from jax import lax
from jax.experimental import pallas as pl
from jax.experimental.pallas import tpu as pltpu

_F32 = jnp.float32
_BF16 = jnp.bfloat16
_U32 = jnp.uint32

SK_S, SK_P, SK_W, W_FIRST = 1, 2, 1, 0


def _make_kernel(S, D, H, Dh, M, seg, F, FC, RB):
    n_pair = S // (2 * seg)
    PR = 2 * seg
    RA = seg - M
    n_fc = F // FC
    n_rb = S // RB
    scale = float(Dh) ** -0.5
    L = M + seg

    def kernel(x_hbm, mem0_ref, wq_hbm, wk_hbm, wv_hbm, wo_hbm, wg_hbm, wu_hbm, wd_hbm,
               out_ref,
               x_v, xn_v, acc_v, wg_b, wu_b, wd_b,
               st_q, st_k, st_v, st_o, wq_p, wk_p, wv_p, wo_p,
               qkv_buf, o_buf, sems):
        def mlp_copies(c, slot):
            c0 = pl.multiple_of(c * FC, FC)
            return (
                pltpu.make_async_copy(wg_hbm.at[:, pl.ds(c0, FC)], wg_b.at[slot], sems.at[0 + slot]),
                pltpu.make_async_copy(wu_hbm.at[:, pl.ds(c0, FC)], wu_b.at[slot], sems.at[2 + slot]),
                pltpu.make_async_copy(wd_hbm.at[pl.ds(c0, FC), :], wd_b.at[slot], sems.at[4 + slot]),
            )
        cp_x = pltpu.make_async_copy(x_hbm, x_v, sems.at[6])
        cp_x.start()
        for cp in mlp_copies(0, 0):
            cp.start()
        cp_a = (
            pltpu.make_async_copy(wq_hbm, st_q, sems.at[7]),
            pltpu.make_async_copy(wk_hbm, st_k, sems.at[8]),
            pltpu.make_async_copy(wv_hbm, st_v, sems.at[9]),
            pltpu.make_async_copy(wo_hbm, st_o, sems.at[10]),
        )
        for cp in cp_a:
            cp.start()

        cp_x.wait()

        def ln_body(r, _):
            r0 = pl.multiple_of(r * 256, 256)
            xv = x_v[pl.ds(r0, 256), :].astype(_F32)
            mu = jnp.mean(xv, axis=-1, keepdims=True)
            xc = xv - mu
            var = jnp.mean(xc * xc, axis=-1, keepdims=True)
            xn_v[pl.ds(r0, 256), :] = (xc * lax.rsqrt(var + 1e-5)).astype(_BF16)
            acc_v[pl.ds(r0, 256), :] = jnp.zeros((256, D), _F32)
            return 0
        lax.fori_loop(0, S // 256, ln_body, 0)

        def mlp_chunk(c, _):
            slot = lax.rem(c, 2)

            @pl.when(c + 1 < n_fc)
            def _():
                for cp in mlp_copies(c + 1, 1 - slot):
                    cp.start()
            for cp in mlp_copies(c, slot):
                cp.wait()

            def rb_body(r, _):
                r0 = pl.multiple_of(r * RB, RB)
                xb = xn_v[pl.ds(r0, RB), :]
                g = jnp.dot(xb, wg_b[slot], preferred_element_type=_F32)
                u = jnp.dot(xb, wu_b[slot], preferred_element_type=_F32)
                h = (jax.nn.sigmoid(g) * u).astype(_BF16)
                acc_v[pl.ds(r0, RB), :] += jnp.dot(h, wd_b[slot], preferred_element_type=_F32)
                return 0
            lax.fori_loop(0, n_rb, rb_body, 0)
            return 0
        lax.fori_loop(0, n_fc, mlp_chunk, 0)

        for cp in cp_a:
            cp.wait()

        def conv3(stage, dst):
            def body(i, _):
                d0 = pl.multiple_of(i * 16, 16)
                v = stage[pl.ds(d0, 16), :, :]
                u = pltpu.bitcast(v, _U32).reshape(8, 2, H // 2, Dh)
                ev = jnp.swapaxes(u[:, 0], 0, 1)
                od = jnp.swapaxes(u[:, 1], 0, 1)
                lo = (ev & jnp.uint32(0xFFFF)) | (od << 16)
                hi = (ev >> 16) | (od & jnp.uint32(0xFFFF0000))
                r0 = pl.multiple_of(i * 8, 8)
                for hp in range(H // 2):
                    dst[2 * hp, pl.ds(r0, 8), :] = lo[hp]
                    dst[2 * hp + 1, pl.ds(r0, 8), :] = hi[hp]
                return 0
            lax.fori_loop(0, D // 16, body, 0)
        conv3(st_q, wq_p)
        conv3(st_k, wk_p)
        conv3(st_v, wv_p)

        def convo(h, _):
            wo_p[h] = pltpu.bitcast(st_o[h], _U32)
            return 0
        lax.fori_loop(0, H, convo, 0)

        def W(ref, h):
            return pltpu.bitcast(ref[h], _BF16)

        x0 = xn_v[pl.ds(0, PR), :]
        for h in range(H):
            for t, wp in enumerate((wq_p, wk_p, wv_p)):
                qkv_buf[0, t * H + h] = jnp.dot(x0, W(wp, h), preferred_element_type=_F32)
        o_buf[1] = jnp.zeros((H, PR, Dh), _F32)

        row = lax.broadcasted_iota(jnp.int32, (L, L), 0)
        col = lax.broadcasted_iota(jnp.int32, (L, L), 1)
        mask = (row < M) | (row >= col)

        def step(mem, cur, nxt, xrow0, seg_off, off, nrows):
            xr = xn_v[pl.ds(xrow0, nrows), :].astype(_F32)
            lhs = jnp.concatenate([mem, xr], axis=0).astype(_BF16)
            acc = None
            qkv, pv, ov = {}, {}, {}
            for t in range(H + SK_S + SK_P + SK_W):
                h = t
                if h < H:
                    qa = jnp.dot(lhs, W(wq_p, h), preferred_element_type=_F32)
                    ka = jnp.dot(lhs, W(wk_p, h), preferred_element_type=_F32)
                    va = jnp.dot(lhs, W(wv_p, h), preferred_element_type=_F32)
                    qkv_buf[nxt, h, pl.ds(off, nrows), :] = qa[M:]
                    qkv_buf[nxt, H + h, pl.ds(off, nrows), :] = ka[M:]
                    qkv_buf[nxt, 2 * H + h, pl.ds(off, nrows), :] = va[M:]
                    q = jnp.concatenate([qa[:M], qkv_buf[cur, h, pl.ds(seg_off, seg), :]], 0).astype(_BF16)
                    k = jnp.concatenate([ka[:M], qkv_buf[cur, H + h, pl.ds(seg_off, seg), :]], 0).astype(_BF16)
                    v = jnp.concatenate([va[:M], qkv_buf[cur, 2 * H + h, pl.ds(seg_off, seg), :]], 0).astype(_BF16)
                    qkv[h] = (q, k, v)
                h = t - SK_S - SK_P - SK_W
                if W_FIRST and 0 <= h < H:
                    part = jnp.dot(ov.pop(h), W(wo_p, h), preferred_element_type=_F32)
                    acc = part if acc is None else acc + part
                h = t - SK_S - SK_P
                if 0 <= h < H:
                    p, v = pv.pop(h)
                    o = jnp.dot(p, v, preferred_element_type=_F32)
                    o_buf[cur, h, pl.ds(seg_off, seg), :] = o[M:]
                    ov[h] = jnp.concatenate([o[:M], o_buf[nxt, h, pl.ds(off, nrows), :]], 0).astype(_BF16)
                h = t - SK_S
                if 0 <= h < H:
                    q, k, v = qkv.pop(h)
                    s = lax.dot_general(q, k, (((1,), (1,)), ((), ())), preferred_element_type=_F32) * scale
                    s = jnp.where(mask, s, -1e9)
                    m = jnp.max(s, axis=-1, keepdims=True)
                    e = jnp.exp(s - m)
                    p = e / jnp.sum(e, axis=-1, keepdims=True)
                    pv[h] = (p.astype(_BF16), v)
                h = t - SK_S - SK_P - SK_W
                if (not W_FIRST) and 0 <= h < H:
                    part = jnp.dot(ov.pop(h), W(wo_p, h), preferred_element_type=_F32)
                    acc = part if acc is None else acc + part
            new_mem = acc[:M].astype(_BF16).astype(_F32)
            return new_mem, acc[M:]

        def finish(r0, nrows, s_rows):
            xv = x_v[pl.ds(r0, nrows), :].astype(_F32)
            gate = jax.nn.silu(acc_v[pl.ds(r0, nrows), :])
            out_ref[pl.ds(r0, nrows), :] = (xv + s_rows * gate).astype(out_ref.dtype)

        def pair_body(j, mem):
            cur = lax.rem(j, 2)
            nxt = 1 - cur
            jn = jnp.minimum(j + 1, n_pair - 1)
            xrow = pl.multiple_of(jn * PR, PR)
            mem, sA = step(mem, cur, nxt, xrow, 0, 0, RA)
            mem, sB = step(mem, cur, nxt, xrow + RA, seg, RA, PR - RA)

            @pl.when(j > 0)
            def _():
                r0 = pl.multiple_of((j - 1) * PR, PR)
                finish(r0, PR, jnp.concatenate([sA, sB], axis=0))
            return mem

        mem = lax.fori_loop(0, n_pair, pair_body, mem0_ref[...].astype(_F32))

        last = (n_pair - 1) % 2
        acc = None
        for h in range(H):
            part = jnp.dot(o_buf[last, h].astype(_BF16), W(wo_p, h), preferred_element_type=_F32)
            acc = part if acc is None else acc + part
        finish(S - PR, PR, acc)

    return kernel


@functools.partial(jax.jit, static_argnames=("A_seg_len",))
def pallas_recurrent_scan__memory_aug_recurrent_mem_tr__glu_gated_glu__prompt_kernel(
        A_x, A_mem0, A_Wq, A_Wk, A_Wv, A_Wo, A_seg_len, B_x, B_w_gate, B_w_up, B_w_down):
    B, S, D = A_x.shape
    assert B == 1
    H, Dh = A_Wq.shape[1], A_Wq.shape[2]
    M = A_mem0.shape[1]
    seg = int(A_seg_len)
    F = B_w_gate.shape[1]
    FC, RB = 512, 512
    PR = 2 * seg
    kernel = _make_kernel(S, D, H, Dh, M, seg, F, FC, RB)
    anyspec = pl.BlockSpec(memory_space=pl.ANY)
    out = pl.pallas_call(
        kernel,
        out_shape=jax.ShapeDtypeStruct((S, D), A_x.dtype),
        in_specs=[anyspec, pl.BlockSpec(memory_space=pltpu.VMEM)] + [anyspec] * 7,
        out_specs=pl.BlockSpec(memory_space=pltpu.VMEM),
        scratch_shapes=[
            pltpu.VMEM((S, D), _BF16), pltpu.VMEM((S, D), _BF16), pltpu.VMEM((S, D), _F32),
            pltpu.VMEM((2, D, FC), _BF16), pltpu.VMEM((2, D, FC), _BF16), pltpu.VMEM((2, FC, D), _BF16),
            pltpu.VMEM((D, H, Dh), _BF16), pltpu.VMEM((D, H, Dh), _BF16), pltpu.VMEM((D, H, Dh), _BF16),
            pltpu.VMEM((H, Dh, D), _BF16),
            pltpu.VMEM((H, D // 2, Dh), _U32), pltpu.VMEM((H, D // 2, Dh), _U32),
            pltpu.VMEM((H, D // 2, Dh), _U32), pltpu.VMEM((H, Dh // 2, D), _U32),
            pltpu.VMEM((2, 3 * H, PR, Dh), _F32), pltpu.VMEM((2, H, PR, Dh), _F32),
            pltpu.SemaphoreType.DMA((11,)),
        ],
        compiler_params=pltpu.CompilerParams(vmem_limit_bytes=120 * 1024 * 1024),
    )(A_x.reshape(S, D), A_mem0.reshape(M, D), A_Wq, A_Wk, A_Wv, A_Wo, B_w_gate, B_w_up, B_w_down)
    return out.reshape(B, S, D)
```

```python
import functools
import numpy as np
import jax
import jax.numpy as jnp
from jax import lax
from jax.experimental import pallas as pl
from jax.experimental.pallas import tpu as pltpu

_F32 = jnp.float32
_BF16 = jnp.bfloat16
_U32 = jnp.uint32
SK_S, SK_P, SK_W, FIN_A, FIN_B = [int(a) for a in '1,3,6,3,3'.split(',')]


def _make_kernel(S, D, H, Dh, M, seg, F, FC, RB):
    n_pair = S // (2 * seg)
    PR = 2 * seg
    RA = seg - M
    n_fc = F // FC
    n_rb = S // RB
    scale = float(Dh) ** -0.5
    L = M + seg
    A_START = int(1)
    C_CONV = int(2)
    n_it = (n_fc - C_CONV) * n_rb
    n_u3 = 3 * D // 16
    U3 = -(-n_u3 // n_it)
    UO = -(-H // n_it)

    def kernel(x_hbm, mem0_ref, wq_hbm, wk_hbm, wv_hbm, wo_hbm, wg_hbm, wu_hbm, wd_hbm,
               out_hbm,
               x_v, xn_v, acc_v, wg_b, wu_b, wd_b,
               st_3, st_o, w3_p, wo_p,
               qkv_buf, o_buf, s_buf, out_v, sems, xsems):
        def mlp_copies(c, slot):
            c0 = pl.multiple_of(c * FC, FC)
            return (
                pltpu.make_async_copy(wg_hbm.at[:, pl.ds(c0, FC)], wg_b.at[slot], sems.at[0 + slot]),
                pltpu.make_async_copy(wu_hbm.at[:, pl.ds(c0, FC)], wu_b.at[slot], sems.at[2 + slot]),
                pltpu.make_async_copy(wd_hbm.at[pl.ds(c0, FC), :], wd_b.at[slot], sems.at[4 + slot]),
            )

        def x_copy(r):
            r0 = pl.multiple_of(r * RB, RB)
            return pltpu.make_async_copy(x_hbm.at[pl.ds(r0, RB), :], x_v.at[pl.ds(r0, RB), :], xsems.at[r])

        x_copy(0).start()
        for cp in mlp_copies(0, 0):
            cp.start()
        cp_a = (
            pltpu.make_async_copy(wq_hbm, st_3.at[pl.ds(0, D)], sems.at[6]),
            pltpu.make_async_copy(wk_hbm, st_3.at[pl.ds(D, D)], sems.at[7]),
            pltpu.make_async_copy(wv_hbm, st_3.at[pl.ds(2 * D, D)], sems.at[8]),
            pltpu.make_async_copy(wo_hbm, st_o, sems.at[9]),
        )
        def ln_block(r):
            for i in range(RB // 256):
                r0 = pl.multiple_of(r * RB + i * 256, 256)
                xv = x_v[pl.ds(r0, 256), :].astype(_F32)
                mu = jnp.mean(xv, axis=-1, keepdims=True)
                xc = xv - mu
                var = jnp.mean(xc * xc, axis=-1, keepdims=True)
                xn_v[pl.ds(r0, 256), :] = (xc * lax.rsqrt(var + 1e-5)).astype(_BF16)

        x_copy(0).wait()
        for r in range(1, n_rb):
            x_copy(r).start()
        for cp in mlp_copies(1, 1):
            cp.start()
        ln_block(0)
        acc_v[...] = jnp.zeros((S, D), _F32)

        def conv3_unit(u):
            m = u // (D // 16)
            i = u - m * (D // 16)
            d0 = pl.multiple_of(u * 16, 16)
            v = st_3[pl.ds(d0, 16), :, :]
            w = pltpu.bitcast(v, _U32).reshape(8, 2, H // 2, Dh)
            ev = jnp.swapaxes(w[:, 0], 0, 1)
            od = jnp.swapaxes(w[:, 1], 0, 1)
            lo = (ev & jnp.uint32(0xFFFF)) | (od << 16)
            hi = (ev >> 16) | (od & jnp.uint32(0xFFFF0000))
            r0 = pl.multiple_of(i * 8, 8)
            for hp in range(H // 2):
                w3_p[m * H + 2 * hp, pl.ds(r0, 8), :] = lo[hp]
                w3_p[m * H + 2 * hp + 1, pl.ds(r0, 8), :] = hi[hp]

        def convo_unit(h):
            wo_p[h] = pltpu.bitcast(st_o[h], _U32)

        def mlp_rows(r, slot):
            r0 = pl.multiple_of(r * RB, RB)
            xb = xn_v[pl.ds(r0, RB), :]
            g = jnp.dot(xb, wg_b[slot], preferred_element_type=_F32)
            u = jnp.dot(xb, wu_b[slot], preferred_element_type=_F32)
            h = (jax.nn.sigmoid(g) * u).astype(_BF16)
            acc_v[pl.ds(r0, RB), :] += jnp.dot(h, wd_b[slot], preferred_element_type=_F32)

        def chunk_head(c):
            slot = lax.rem(c, 2)

            @pl.when(jnp.logical_and(c + 1 < n_fc, c >= 1))
            def _():
                for cp in mlp_copies(c + 1, 1 - slot):
                    cp.start()
            for cp in mlp_copies(c, slot):
                cp.wait()
            return slot

        def chunk_ln(c, _):
            slot = chunk_head(c)

            def rb_body(r, _):
                rn = jnp.minimum(r + 1, n_rb - 1)

                @pl.when(jnp.logical_and(c == 0, r + 1 < n_rb))
                def _():
                    x_copy(rn).wait()

                @pl.when(jnp.logical_and(c == 0, r == A_START))
                def _():
                    for cp in cp_a:
                        cp.start()
                mlp_rows(r, slot)
                ln_block(rn)
                return 0
            lax.fori_loop(0, n_rb, rb_body, 0)
            return 0
        lax.fori_loop(0, C_CONV, chunk_ln, 0)

        for cp in cp_a:
            cp.wait()

        def chunk_conv(c, _):
            slot = chunk_head(c)

            def rb_body(r, _):
                it = (c - C_CONV) * n_rb + r
                mlp_rows(r, slot)
                for k in range(U3):
                    conv3_unit(jnp.minimum(it * U3 + k, n_u3 - 1))
                for k in range(UO):
                    convo_unit(jnp.minimum(it * UO + k, H - 1))
                return 0
            lax.fori_loop(0, n_rb, rb_body, 0)
            return 0
        lax.fori_loop(C_CONV, n_fc, chunk_conv, 0)

        def W3(t, h):
            return pltpu.bitcast(w3_p[t * H + h], _BF16)

        def WO(h):
            return pltpu.bitcast(wo_p[h], _BF16)

        x0 = xn_v[pl.ds(0, PR), :]
        for h in range(H):
            for t in range(3):
                qkv_buf[0, t * H + h] = jnp.dot(x0, W3(t, h), preferred_element_type=_F32)
        o_buf[1] = jnp.zeros((H, PR, Dh), _F32)
        s_buf[...] = jnp.zeros((PR, D), _F32)

        row = lax.broadcasted_iota(jnp.int32, (L, L), 0)
        col = lax.broadcasted_iota(jnp.int32, (L, L), 1)
        mask = (row < M) | (row >= col)

        def finish(r0, nrows, s_rows):
            xv = x_v[pl.ds(r0, nrows), :].astype(_F32)
            gate = jax.nn.silu(acc_v[pl.ds(r0, nrows), :])
            out_v[pl.ds(r0, nrows), :] = (xv + s_rows * gate).astype(out_v.dtype)

        def out_copy(p):
            r0 = pl.multiple_of(p * PR, PR)
            return pltpu.make_async_copy(out_v.at[pl.ds(r0, PR), :], out_hbm.at[pl.ds(r0, PR), :], sems.at[10])

        def step(mem, cur, nxt, xrow0, seg_off, off, nrows, extra, t_extra):
            xr = xn_v[pl.ds(xrow0, nrows), :].astype(_F32)
            lhs = jnp.concatenate([mem, xr], axis=0).astype(_BF16)
            acc = None
            qkv, pv, ov = {}, {}, {}
            for t in range(H + SK_S + SK_P + SK_W):
                h = t
                if h < H:
                    qa = jnp.dot(lhs, W3(0, h), preferred_element_type=_F32)
                    ka = jnp.dot(lhs, W3(1, h), preferred_element_type=_F32)
                    va = jnp.dot(lhs, W3(2, h), preferred_element_type=_F32)
                    qkv_buf[nxt, h, pl.ds(off, nrows), :] = qa[M:]
                    qkv_buf[nxt, H + h, pl.ds(off, nrows), :] = ka[M:]
                    qkv_buf[nxt, 2 * H + h, pl.ds(off, nrows), :] = va[M:]
                    q = jnp.concatenate([qa[:M], qkv_buf[cur, h, pl.ds(seg_off, seg), :]], 0).astype(_BF16)
                    k = jnp.concatenate([ka[:M], qkv_buf[cur, H + h, pl.ds(seg_off, seg), :]], 0).astype(_BF16)
                    v = jnp.concatenate([va[:M], qkv_buf[cur, 2 * H + h, pl.ds(seg_off, seg), :]], 0).astype(_BF16)
                    qkv[h] = (q, k, v)
                if t == t_extra:
                    extra()
                h = t - SK_S - SK_P
                if 0 <= h < H:
                    p, v = pv.pop(h)
                    o = jnp.dot(p, v, preferred_element_type=_F32)
                    o_buf[cur, h, pl.ds(seg_off, seg), :] = o[M:]
                    ov[h] = jnp.concatenate([o[:M], o_buf[nxt, h, pl.ds(off, nrows), :]], 0).astype(_BF16)
                h = t - SK_S
                if 0 <= h < H:
                    q, k, v = qkv.pop(h)
                    s = lax.dot_general(q, k, (((1,), (1,)), ((), ())), preferred_element_type=_F32) * scale
                    s = jnp.where(mask, s, -1e9)
                    m = jnp.max(s, axis=-1, keepdims=True)
                    e = jnp.exp(s - m)
                    p = e / jnp.sum(e, axis=-1, keepdims=True)
                    pv[h] = (p.astype(_BF16), v)
                h = t - SK_S - SK_P - SK_W
                if 0 <= h < H:
                    part = jnp.dot(ov.pop(h), WO(h), preferred_element_type=_F32)
                    acc = part if acc is None else acc + part
            new_mem = acc[:M].astype(_BF16).astype(_F32)
            return new_mem, acc[M:]

        def pair_body(j, mem):
            cur = lax.rem(j, 2)
            nxt = 1 - cur
            jn = jnp.minimum(j + 1, n_pair - 1)
            xrow = pl.multiple_of(jn * PR, PR)
            rp2 = pl.multiple_of(jnp.maximum(j - 2, 0) * PR, PR)
            rp1 = pl.multiple_of(jnp.maximum(j - 1, 0) * PR, PR)

            def fin_b():
                finish(rp2 + RA, PR - RA, s_buf[pl.ds(RA, PR - RA), :])
            mem, sA = step(mem, cur, nxt, xrow, 0, 0, RA, fin_b, FIN_A)

            def fin_a():
                finish(rp1, RA, sA)
            mem, sB = step(mem, cur, nxt, xrow + RA, seg, RA, PR - RA, fin_a, FIN_B)
            s_buf[pl.ds(RA, PR - RA), :] = sB

            @pl.when(j >= 2)
            def _():
                out_copy(j - 2).start()
            return mem

        mem = lax.fori_loop(0, n_pair, pair_body, mem0_ref[...].astype(_F32))

        finish(S - 2 * PR + RA, PR - RA, s_buf[pl.ds(RA, PR - RA), :])
        out_copy(n_pair - 2).start()
        last = (n_pair - 1) % 2
        acc = None
        for h in range(H):
            part = jnp.dot(o_buf[last, h].astype(_BF16), WO(h), preferred_element_type=_F32)
            acc = part if acc is None else acc + part
        finish(S - PR, PR, acc)
        out_copy(n_pair - 1).start()
        for p in range(n_pair):
            out_copy(p).wait()

    return kernel


@functools.partial(jax.jit, static_argnames=("A_seg_len",))
def pallas_recurrent_scan__memory_aug_recurrent_mem_tr__glu_gated_glu__prompt_kernel(
        A_x, A_mem0, A_Wq, A_Wk, A_Wv, A_Wo, A_seg_len, B_x, B_w_gate, B_w_up, B_w_down):
    B, S, D = A_x.shape
    assert B == 1
    H, Dh = A_Wq.shape[1], A_Wq.shape[2]
    M = A_mem0.shape[1]
    seg = int(A_seg_len)
    F = B_w_gate.shape[1]
    FC, RB = 512, 512
    PR = 2 * seg
    kernel = _make_kernel(S, D, H, Dh, M, seg, F, FC, RB)
    anyspec = pl.BlockSpec(memory_space=pl.ANY)
    out = pl.pallas_call(
        kernel,
        out_shape=jax.ShapeDtypeStruct((S, D), A_x.dtype),
        in_specs=[anyspec, pl.BlockSpec(memory_space=pltpu.VMEM)] + [anyspec] * 7,
        out_specs=anyspec,
        scratch_shapes=[
            pltpu.VMEM((S, D), _BF16), pltpu.VMEM((S, D), _BF16), pltpu.VMEM((S, D), _F32),
            pltpu.VMEM((2, D, FC), _BF16), pltpu.VMEM((2, D, FC), _BF16), pltpu.VMEM((2, FC, D), _BF16),
            pltpu.VMEM((3 * D, H, Dh), _BF16), pltpu.VMEM((H, Dh, D), _BF16),
            pltpu.VMEM((3 * H, D // 2, Dh), _U32), pltpu.VMEM((H, Dh // 2, D), _U32),
            pltpu.VMEM((2, 3 * H, PR, Dh), _F32), pltpu.VMEM((2, H, PR, Dh), _F32),
            pltpu.VMEM((PR, D), _F32), pltpu.VMEM((S, D), _BF16),
            pltpu.SemaphoreType.DMA((11,)), pltpu.SemaphoreType.DMA((S // RB,)),
        ],
        compiler_params=pltpu.CompilerParams(vmem_limit_bytes=120 * 1024 * 1024),
    )(A_x.reshape(S, D), A_mem0.reshape(M, D), A_Wq, A_Wk, A_Wv, A_Wo, B_w_gate, B_w_up, B_w_down)
    return out.reshape(B, S, D)
```

```python
import functools
import numpy as np
import jax
import jax.numpy as jnp
from jax import lax
from jax.experimental import pallas as pl
from jax.experimental.pallas import tpu as pltpu

_F32 = jnp.float32
_BF16 = jnp.bfloat16
_U32 = jnp.uint32
SK_S, SK_P, SK_W, FIN_A, FIN_B = [int(a) for a in '1,6,4,3,3'.split(',')]


def _make_kernel(S, D, H, Dh, M, seg, F, FC, RB):
    n_pair = S // (2 * seg)
    PR = 2 * seg
    RA = seg - M
    n_fc = F // FC
    n_rb = S // RB
    scale = float(Dh) ** -0.5
    L = M + seg
    UNR = int(1)
    A_START = int('1')
    C_CONV = int(2)
    n_it = (n_fc - C_CONV) * n_rb
    n_u3 = 3 * D // 16
    U3 = -(-n_u3 // n_it)
    UO = -(-H // n_it)

    def kernel(x_hbm, mem0_ref, wq_hbm, wk_hbm, wv_hbm, wo_hbm, wg_hbm, wu_hbm, wd_hbm,
               out_hbm,
               x_v, xn_v, acc_v, wg_b, wu_b, wd_b,
               w3_p, wo_p,
               qkv_buf, o_buf, s_buf, out_v, sems, xsems):
        def mlp_copies(c, slot):
            c0 = pl.multiple_of(c * FC, FC)
            return (
                pltpu.make_async_copy(wg_hbm.at[:, pl.ds(c0, FC)], wg_b.at[slot], sems.at[0 + slot]),
                pltpu.make_async_copy(wu_hbm.at[:, pl.ds(c0, FC)], wu_b.at[slot], sems.at[2 + slot]),
                pltpu.make_async_copy(wd_hbm.at[pl.ds(c0, FC), :], wd_b.at[slot], sems.at[4 + slot]),
            )

        def x_copy(r):
            r0 = pl.multiple_of(r * RB, RB)
            return pltpu.make_async_copy(x_hbm.at[pl.ds(r0, RB), :], x_v.at[pl.ds(r0, RB), :], xsems.at[r])

        x_copy(0).start()
        for cp in mlp_copies(0, 0):
            cp.start()
        def a_copies(part):
            cps = []
            for t, w_hbm in enumerate((wq_hbm, wk_hbm, wv_hbm)):
                if t != part:
                    continue
                w32 = w_hbm.bitcast(_U32)
                for hp in range(H // 2):
                    for par in range(2):
                        cps.append(pltpu.make_async_copy(w32.at[:, par, hp, :], w3_p.at[t * H + 2 * hp + par], sems.at[6]))
            if part == 3:
                cps.append(pltpu.make_async_copy(wo_hbm.bitcast(_U32), wo_p, sems.at[7]))
            return cps

        def ln_block(r):
            for i in range(RB // 256):
                r0 = pl.multiple_of(r * RB + i * 256, 256)
                xv = x_v[pl.ds(r0, 256), :].astype(_F32)
                mu = jnp.mean(xv, axis=-1, keepdims=True)
                xc = xv - mu
                var = jnp.mean(xc * xc, axis=-1, keepdims=True)
                xn_v[pl.ds(r0, 256), :] = (xc * lax.rsqrt(var + 1e-5)).astype(_BF16)

        acc_v[...] = jnp.zeros((S, D), _F32)
        x_copy(0).wait()
        for r in range(1, n_rb):
            x_copy(r).start()
        for cp in mlp_copies(1, 1):
            cp.start()
        ln_block(0)

        def mlp_rows(r, slot):
            r0 = pl.multiple_of(r * RB, RB)
            xb = xn_v[pl.ds(r0, RB), :]
            g = jnp.dot(xb, wg_b[slot], preferred_element_type=_F32)
            u = jnp.dot(xb, wu_b[slot], preferred_element_type=_F32)
            h = (jax.nn.sigmoid(g) * u).astype(_BF16)
            acc_v[pl.ds(r0, RB), :] += jnp.dot(h, wd_b[slot], preferred_element_type=_F32)

        def chunk_head(c):
            slot = lax.rem(c, 2)

            @pl.when(jnp.logical_and(c + 1 < n_fc, c >= 1))
            def _():
                for cp in mlp_copies(c + 1, 1 - slot):
                    cp.start()
            for cp in mlp_copies(c, slot):
                cp.wait()

        chunk_head(0)

        def ln_body(r, _):
            x_copy(r + 1).wait()

            mlp_rows(r, 0)
            ln_block(r + 1)
            return 0
        lax.fori_loop(0, n_rb - 1, ln_body, 0)

        def mlp_body(it, _):
            c = it // n_rb
            r = it - c * n_rb

            @pl.when(r == 0)
            def _():
                chunk_head(c)
                for part in range(4):
                    @pl.when(c == part + A_START)
                    def _():
                        for cp in a_copies(part):
                            cp.start()
            mlp_rows(r, lax.rem(c, 2))
            return 0
        lax.fori_loop(n_rb - 1, n_fc * n_rb, mlp_body, 0)

        for part in range(4):
            for cp in a_copies(part):
                cp.wait()

        def W3(t, h):
            return pltpu.bitcast(w3_p[t * H + h], _BF16)

        def WO(h):
            return pltpu.bitcast(wo_p[h], _BF16)

        x0 = xn_v[pl.ds(0, PR), :]
        for hp in range(H // 2):
            for t in range(3):
                ev = w3_p[t * H + 2 * hp]
                od = w3_p[t * H + 2 * hp + 1]
                lo = (ev & jnp.uint32(0xFFFF)) | (od << 16)
                hi = (ev >> 16) | (od & jnp.uint32(0xFFFF0000))
                w3_p[t * H + 2 * hp] = lo
                w3_p[t * H + 2 * hp + 1] = hi
                qkv_buf[0, t * H + 2 * hp] = jnp.dot(x0, pltpu.bitcast(lo, _BF16), preferred_element_type=_F32)
                qkv_buf[0, t * H + 2 * hp + 1] = jnp.dot(x0, pltpu.bitcast(hi, _BF16), preferred_element_type=_F32)
        o_buf[1] = jnp.zeros((H, PR, Dh), _F32)
        s_buf[...] = jnp.zeros((PR, D), _F32)

        row = lax.broadcasted_iota(jnp.int32, (L, L), 0)
        col = lax.broadcasted_iota(jnp.int32, (L, L), 1)
        mask = (row < M) | (row >= col)

        def finish(r0, nrows, s_rows):
            xv = x_v[pl.ds(r0, nrows), :].astype(_F32)
            gate = jax.nn.silu(acc_v[pl.ds(r0, nrows), :])
            out_v[pl.ds(r0, nrows), :] = (xv + s_rows * gate).astype(out_v.dtype)

        def out_copy(p):
            r0 = pl.multiple_of(p * PR, PR)
            return pltpu.make_async_copy(out_v.at[pl.ds(r0, PR), :], out_hbm.at[pl.ds(r0, PR), :], sems.at[10])

        def step(mem, cur, nxt, xrow0, seg_off, off, nrows, extra, t_extra):
            xr = xn_v[pl.ds(xrow0, nrows), :].astype(_F32)
            lhs = jnp.concatenate([mem, xr], axis=0).astype(_BF16)
            acc = None
            qkv, pv, ov = {}, {}, {}
            for t in range(H + SK_S + SK_P + SK_W):
                h = t
                if h < H:
                    qa = jnp.dot(lhs, W3(0, h), preferred_element_type=_F32)
                    ka = jnp.dot(lhs, W3(1, h), preferred_element_type=_F32)
                    va = jnp.dot(lhs, W3(2, h), preferred_element_type=_F32)
                    qkv_buf[nxt, h, pl.ds(off, nrows), :] = qa[M:]
                    qkv_buf[nxt, H + h, pl.ds(off, nrows), :] = ka[M:]
                    qkv_buf[nxt, 2 * H + h, pl.ds(off, nrows), :] = va[M:]
                    q = jnp.concatenate([qa[:M], qkv_buf[cur, h, pl.ds(seg_off, seg), :]], 0).astype(_BF16)
                    k = jnp.concatenate([ka[:M], qkv_buf[cur, H + h, pl.ds(seg_off, seg), :]], 0).astype(_BF16)
                    v = jnp.concatenate([va[:M], qkv_buf[cur, 2 * H + h, pl.ds(seg_off, seg), :]], 0).astype(_BF16)
                    qkv[h] = (q, k, v)
                if t == t_extra:
                    extra()
                h = t - SK_S - SK_P
                if 0 <= h < H:
                    p, v = pv.pop(h)
                    o = jnp.dot(p, v, preferred_element_type=_F32)
                    o_buf[cur, h, pl.ds(seg_off, seg), :] = o[M:]
                    ov[h] = jnp.concatenate([o[:M], o_buf[nxt, h, pl.ds(off, nrows), :]], 0).astype(_BF16)
                h = t - SK_S
                if 0 <= h < H:
                    q, k, v = qkv.pop(h)
                    s = lax.dot_general(q, k, (((1,), (1,)), ((), ())), preferred_element_type=_F32) * scale
                    s = jnp.where(mask, s, -1e9)
                    m = jnp.max(s, axis=-1, keepdims=True)
                    e = jnp.exp(s - m)
                    p = e / jnp.sum(e, axis=-1, keepdims=True)
                    pv[h] = (p.astype(_BF16), v)
                h = t - SK_S - SK_P - SK_W
                if 0 <= h < H:
                    part = jnp.dot(ov.pop(h), WO(h), preferred_element_type=_F32)
                    acc = part if acc is None else acc + part
            new_mem = acc[:M].astype(_BF16).astype(_F32)
            return new_mem, acc[M:]

        def pair_body(j, mem):
            cur = lax.rem(j, 2)
            nxt = 1 - cur
            jn = jnp.minimum(j + 1, n_pair - 1)
            xrow = pl.multiple_of(jn * PR, PR)
            rp2 = pl.multiple_of(jnp.maximum(j - 2, 0) * PR, PR)
            rp1 = pl.multiple_of(jnp.maximum(j - 1, 0) * PR, PR)

            def fin_b():
                finish(rp2 + RA, PR - RA, s_buf[pl.ds(RA, PR - RA), :])
            mem, sA = step(mem, cur, nxt, xrow, 0, 0, RA, fin_b, FIN_A)

            def fin_a():
                finish(rp1, RA, sA)
            mem, sB = step(mem, cur, nxt, xrow + RA, seg, RA, PR - RA, fin_a, FIN_B)
            s_buf[pl.ds(RA, PR - RA), :] = sB

            @pl.when(j >= 2)
            def _():
                out_copy(j - 2).start()
            return mem

        mem = lax.fori_loop(0, n_pair, pair_body, mem0_ref[...].astype(_F32), unroll=UNR)

        finish(S - 2 * PR + RA, PR - RA, s_buf[pl.ds(RA, PR - RA), :])
        out_copy(n_pair - 2).start()
        last = (n_pair - 1) % 2
        acc = None
        for h in range(H):
            part = jnp.dot(o_buf[last, h].astype(_BF16), WO(h), preferred_element_type=_F32)
            acc = part if acc is None else acc + part
        finish(S - PR, PR, acc)
        out_copy(n_pair - 1).start()
        for p in range(n_pair):
            out_copy(p).wait()

    return kernel


@functools.partial(jax.jit, static_argnames=("A_seg_len",))
def pallas_recurrent_scan__memory_aug_recurrent_mem_tr__glu_gated_glu__prompt_kernel(
        A_x, A_mem0, A_Wq, A_Wk, A_Wv, A_Wo, A_seg_len, B_x, B_w_gate, B_w_up, B_w_down):
    B, S, D = A_x.shape
    assert B == 1
    H, Dh = A_Wq.shape[1], A_Wq.shape[2]
    M = A_mem0.shape[1]
    seg = int(A_seg_len)
    F = B_w_gate.shape[1]
    FC, RB = int(512), int('256')
    PR = 2 * seg
    kernel = _make_kernel(S, D, H, Dh, M, seg, F, FC, RB)
    anyspec = pl.BlockSpec(memory_space=pl.ANY)
    out = pl.pallas_call(
        kernel,
        out_shape=jax.ShapeDtypeStruct((S, D), A_x.dtype),
        in_specs=[anyspec, pl.BlockSpec(memory_space=pltpu.VMEM)] + [anyspec] * 7,
        out_specs=anyspec,
        scratch_shapes=[
            pltpu.VMEM((S, D), _BF16), pltpu.VMEM((S, D), _BF16), pltpu.VMEM((S, D), _F32),
            pltpu.VMEM((2, D, FC), _BF16), pltpu.VMEM((2, D, FC), _BF16), pltpu.VMEM((2, FC, D), _BF16),
            pltpu.VMEM((3 * H, D // 2, Dh), _U32), pltpu.VMEM((H, Dh // 2, D), _U32),
            pltpu.VMEM((2, 3 * H, PR, Dh), _F32), pltpu.VMEM((2, H, PR, Dh), _F32),
            pltpu.VMEM((PR, D), _F32), pltpu.VMEM((S, D), _BF16),
            pltpu.SemaphoreType.DMA((11,)), pltpu.SemaphoreType.DMA((S // RB,)),
        ],
        compiler_params=pltpu.CompilerParams(vmem_limit_bytes=120 * 1024 * 1024),
    )(A_x.reshape(S, D), A_mem0.reshape(M, D), A_Wq.reshape(D // 2, 2, H, Dh), A_Wk.reshape(D // 2, 2, H, Dh),
      A_Wv.reshape(D // 2, 2, H, Dh), A_Wo, B_w_gate, B_w_up, B_w_down)
    return out.reshape(B, S, D)
```

```python
import functools
import numpy as np
import jax
import jax.numpy as jnp
from jax import lax
from jax.experimental import pallas as pl
from jax.experimental.pallas import tpu as pltpu

_F32 = jnp.float32
_BF16 = jnp.bfloat16
_U32 = jnp.uint32
SK_S, SK_P, SK_W, FIN_A, FIN_B = [int(a) for a in '1,6,4,3,3'.split(',')]


def _make_kernel(S, D, H, Dh, M, seg, F, FC, RB):
    n_pair = S // (2 * seg)
    PR = 2 * seg
    RA = seg - M
    n_fc = F // FC
    n_rb = S // RB
    scale = float(Dh) ** -0.5
    L = M + seg
    UNR = int(1)
    C_CONV = int('2')
    n_it = (n_fc - C_CONV) * n_rb
    n_u3 = 3 * D // 16
    U3 = -(-n_u3 // n_it)
    UO = -(-H // n_it)

    def kernel(x_hbm, mem0_ref, wq_hbm, wk_hbm, wv_hbm, wo_hbm, wg_hbm, wu_hbm, wd_hbm,
               out_hbm,
               x_v, xn_v, acc_v, wg_b, wu_b, wd_b,
               st_3, st_o, w3_p, wo_p,
               qkv_buf, o_buf, s_buf, out_v, sems, xsems):
        def mlp_copies(c, slot):
            c0 = pl.multiple_of(c * FC, FC)
            return (
                pltpu.make_async_copy(wg_hbm.at[:, pl.ds(c0, FC)], wg_b.at[slot], sems.at[0 + slot]),
                pltpu.make_async_copy(wu_hbm.at[:, pl.ds(c0, FC)], wu_b.at[slot], sems.at[2 + slot]),
                pltpu.make_async_copy(wd_hbm.at[pl.ds(c0, FC), :], wd_b.at[slot], sems.at[4 + slot]),
            )

        def x_copy(r):
            r0 = pl.multiple_of(r * RB, RB)
            return pltpu.make_async_copy(x_hbm.at[pl.ds(r0, RB), :], x_v.at[pl.ds(r0, RB), :], xsems.at[r])

        x_copy(0).start()
        for cp in mlp_copies(0, 0):
            cp.start()
        def a_copies(part):
            if part == 3:
                return [pltpu.make_async_copy(wo_hbm, st_o, sems.at[9])]
            w_hbm = (wq_hbm, wk_hbm, wv_hbm)[part]
            return [pltpu.make_async_copy(w_hbm, st_3.at[pl.ds(part * D, D)], sems.at[6 + part])]

        def ln_block(r):
            for i in range(RB // 256):
                r0 = pl.multiple_of(r * RB + i * 256, 256)
                xv = x_v[pl.ds(r0, 256), :].astype(_F32)
                mu = jnp.mean(xv, axis=-1, keepdims=True)
                xc = xv - mu
                var = jnp.mean(xc * xc, axis=-1, keepdims=True)
                xn_v[pl.ds(r0, 256), :] = (xc * lax.rsqrt(var + 1e-5)).astype(_BF16)

        acc_v[...] = jnp.zeros((S, D), _F32)
        x_copy(0).wait()
        for r in range(1, n_rb):
            x_copy(r).start()
        for cp in mlp_copies(1, 1):
            cp.start()
        ln_block(0)

        def mlp_rows(r, slot):
            r0 = pl.multiple_of(r * RB, RB)
            xb = xn_v[pl.ds(r0, RB), :]
            g = jnp.dot(xb, wg_b[slot], preferred_element_type=_F32)
            u = jnp.dot(xb, wu_b[slot], preferred_element_type=_F32)
            h = (jax.nn.sigmoid(g) * u).astype(_BF16)
            acc_v[pl.ds(r0, RB), :] += jnp.dot(h, wd_b[slot], preferred_element_type=_F32)

        def chunk_head(c):
            slot = lax.rem(c, 2)

            @pl.when(jnp.logical_and(c + 1 < n_fc, c >= 1))
            def _():
                for cp in mlp_copies(c + 1, 1 - slot):
                    cp.start()
            for cp in mlp_copies(c, slot):
                cp.wait()

        chunk_head(0)

        def ln_body(r, _):
            x_copy(r + 1).wait()

            @pl.when(r == 0)
            def _():
                for part in range(4):
                    for cp in a_copies(part):
                        cp.start()

            mlp_rows(r, 0)
            ln_block(r + 1)
            return 0
        lax.fori_loop(0, n_rb - 1, ln_body, 0)

        def conv3_unit(u):
            m = u // (D // 16)
            i = u - m * (D // 16)
            v = st_3[pl.ds(pl.multiple_of(u * 16, 16), 16), :, :]
            w = pltpu.bitcast(v, _U32).reshape(8, 2, H // 2, Dh)
            ev = jnp.swapaxes(w[:, 0], 0, 1)
            od = jnp.swapaxes(w[:, 1], 0, 1)
            lo = (ev & jnp.uint32(0xFFFF)) | (od << 16)
            hi = (ev >> 16) | (od & jnp.uint32(0xFFFF0000))
            r0 = pl.multiple_of(i * 8, 8)
            for hp in range(H // 2):
                w3_p[m * H + 2 * hp, pl.ds(r0, 8), :] = lo[hp]
                w3_p[m * H + 2 * hp + 1, pl.ds(r0, 8), :] = hi[hp]

        def mlp_body(it, _, conv=False):
            c = it // n_rb
            r = it - c * n_rb

            @pl.when(r == 0)
            def _():
                chunk_head(c)
            mlp_rows(r, lax.rem(c, 2))
            if conv:
                k0 = it - C_CONV * n_rb
                for k in range(U3):
                    conv3_unit(jnp.minimum(k0 * U3 + k, n_u3 - 1))
                for k in range(UO):
                    hh = jnp.minimum(k0 * UO + k, H - 1)
                    wo_p[hh] = pltpu.bitcast(st_o[hh], _U32)
            return 0
        lax.fori_loop(n_rb - 1, C_CONV * n_rb, mlp_body, 0)
        for part in range(4):
            for cp in a_copies(part):
                cp.wait()
        lax.fori_loop(C_CONV * n_rb, n_fc * n_rb, functools.partial(mlp_body, conv=True), 0)

        def W3(t, h):
            return pltpu.bitcast(w3_p[t * H + h], _BF16)

        def WO(h):
            return pltpu.bitcast(wo_p[h], _BF16)

        x0 = xn_v[pl.ds(0, PR), :]
        for h in range(H):
            for t in range(3):
                qkv_buf[0, t * H + h] = jnp.dot(x0, W3(t, h), preferred_element_type=_F32)
        o_buf[1] = jnp.zeros((H, PR, Dh), _F32)
        s_buf[...] = jnp.zeros((PR, D), _F32)

        row = lax.broadcasted_iota(jnp.int32, (L, L), 0)
        col = lax.broadcasted_iota(jnp.int32, (L, L), 1)
        mask = (row < M) | (row >= col)

        def finish(r0, nrows, s_rows):
            xv = x_v[pl.ds(r0, nrows), :].astype(_F32)
            gate = jax.nn.silu(acc_v[pl.ds(r0, nrows), :])
            out_v[pl.ds(r0, nrows), :] = (xv + s_rows * gate).astype(out_v.dtype)

        def out_copy(p):
            r0 = pl.multiple_of(p * PR, PR)
            return pltpu.make_async_copy(out_v.at[pl.ds(r0, PR), :], out_hbm.at[pl.ds(r0, PR), :], sems.at[10])

        def step(mem, cur, nxt, xrow0, seg_off, off, nrows, extra, t_extra):
            xr = xn_v[pl.ds(xrow0, nrows), :].astype(_F32)
            lhs = jnp.concatenate([mem, xr], axis=0).astype(_BF16)
            acc = None
            qkv, pv, ov = {}, {}, {}
            for t in range(H + SK_S + SK_P + SK_W):
                h = t
                if h < H:
                    qa = jnp.dot(lhs, W3(0, h), preferred_element_type=_F32)
                    ka = jnp.dot(lhs, W3(1, h), preferred_element_type=_F32)
                    va = jnp.dot(lhs, W3(2, h), preferred_element_type=_F32)
                    qkv_buf[nxt, h, pl.ds(off, nrows), :] = qa[M:]
                    qkv_buf[nxt, H + h, pl.ds(off, nrows), :] = ka[M:]
                    qkv_buf[nxt, 2 * H + h, pl.ds(off, nrows), :] = va[M:]
                    q = jnp.concatenate([qa[:M], qkv_buf[cur, h, pl.ds(seg_off, seg), :]], 0).astype(_BF16)
                    k = jnp.concatenate([ka[:M], qkv_buf[cur, H + h, pl.ds(seg_off, seg), :]], 0).astype(_BF16)
                    v = jnp.concatenate([va[:M], qkv_buf[cur, 2 * H + h, pl.ds(seg_off, seg), :]], 0).astype(_BF16)
                    qkv[h] = (q, k, v)
                if t == t_extra:
                    extra()
                h = t - SK_S - SK_P
                if 0 <= h < H:
                    p, v = pv.pop(h)
                    o = jnp.dot(p, v, preferred_element_type=_F32)
                    o_buf[cur, h, pl.ds(seg_off, seg), :] = o[M:]
                    ov[h] = jnp.concatenate([o[:M], o_buf[nxt, h, pl.ds(off, nrows), :]], 0).astype(_BF16)
                h = t - SK_S
                if 0 <= h < H:
                    q, k, v = qkv.pop(h)
                    s = lax.dot_general(q, k, (((1,), (1,)), ((), ())), preferred_element_type=_F32) * scale
                    s = jnp.where(mask, s, -1e9)
                    m = jnp.max(s, axis=-1, keepdims=True)
                    e = jnp.exp(s - m)
                    p = e / jnp.sum(e, axis=-1, keepdims=True)
                    pv[h] = (p.astype(_BF16), v)
                h = t - SK_S - SK_P - SK_W
                if 0 <= h < H:
                    part = jnp.dot(ov.pop(h), WO(h), preferred_element_type=_F32)
                    acc = part if acc is None else acc + part
            new_mem = acc[:M].astype(_BF16).astype(_F32)
            return new_mem, acc[M:]

        def pair_body(j, mem):
            cur = lax.rem(j, 2)
            nxt = 1 - cur
            jn = jnp.minimum(j + 1, n_pair - 1)
            xrow = pl.multiple_of(jn * PR, PR)
            rp2 = pl.multiple_of(jnp.maximum(j - 2, 0) * PR, PR)
            rp1 = pl.multiple_of(jnp.maximum(j - 1, 0) * PR, PR)

            def fin_b():
                finish(rp2 + RA, PR - RA, s_buf[pl.ds(RA, PR - RA), :])
            mem, sA = step(mem, cur, nxt, xrow, 0, 0, RA, fin_b, FIN_A)

            def fin_a():
                finish(rp1, RA, sA)
            mem, sB = step(mem, cur, nxt, xrow + RA, seg, RA, PR - RA, fin_a, FIN_B)
            s_buf[pl.ds(RA, PR - RA), :] = sB

            @pl.when(j >= 2)
            def _():
                out_copy(j - 2).start()
            return mem

        mem = lax.fori_loop(0, n_pair, pair_body, mem0_ref[...].astype(_F32), unroll=UNR)

        finish(S - 2 * PR + RA, PR - RA, s_buf[pl.ds(RA, PR - RA), :])
        out_copy(n_pair - 2).start()
        last = (n_pair - 1) % 2
        acc = None
        for h in range(H):
            part = jnp.dot(o_buf[last, h].astype(_BF16), WO(h), preferred_element_type=_F32)
            acc = part if acc is None else acc + part
        finish(S - PR, PR, acc)
        out_copy(n_pair - 1).start()
        for p in range(n_pair):
            out_copy(p).wait()

    return kernel


@functools.partial(jax.jit, static_argnames=("A_seg_len",))
def pallas_recurrent_scan__memory_aug_recurrent_mem_tr__glu_gated_glu__prompt_kernel(
        A_x, A_mem0, A_Wq, A_Wk, A_Wv, A_Wo, A_seg_len, B_x, B_w_gate, B_w_up, B_w_down):
    B, S, D = A_x.shape
    assert B == 1
    H, Dh = A_Wq.shape[1], A_Wq.shape[2]
    M = A_mem0.shape[1]
    seg = int(A_seg_len)
    F = B_w_gate.shape[1]
    FC, RB = int(512), int('512')
    PR = 2 * seg
    kernel = _make_kernel(S, D, H, Dh, M, seg, F, FC, RB)
    anyspec = pl.BlockSpec(memory_space=pl.ANY)
    out = pl.pallas_call(
        kernel,
        out_shape=jax.ShapeDtypeStruct((S, D), A_x.dtype),
        in_specs=[anyspec, pl.BlockSpec(memory_space=pltpu.VMEM)] + [anyspec] * 7,
        out_specs=anyspec,
        scratch_shapes=[
            pltpu.VMEM((S, D), _BF16), pltpu.VMEM((S, D), _BF16), pltpu.VMEM((S, D), _F32),
            pltpu.VMEM((2, D, FC), _BF16), pltpu.VMEM((2, D, FC), _BF16), pltpu.VMEM((2, FC, D), _BF16),
            pltpu.VMEM((3 * D, H, Dh), _BF16), pltpu.VMEM((H, Dh, D), _BF16),
            pltpu.VMEM((3 * H, D // 2, Dh), _U32), pltpu.VMEM((H, Dh // 2, D), _U32),
            pltpu.VMEM((2, 3 * H, PR, Dh), _F32), pltpu.VMEM((2, H, PR, Dh), _F32),
            pltpu.VMEM((PR, D), _F32), pltpu.VMEM((S, D), _BF16),
            pltpu.SemaphoreType.DMA((11,)), pltpu.SemaphoreType.DMA((S // RB,)),
        ],
        compiler_params=pltpu.CompilerParams(vmem_limit_bytes=120 * 1024 * 1024),
    )(A_x.reshape(S, D), A_mem0.reshape(M, D), A_Wq, A_Wk, A_Wv, A_Wo, B_w_gate, B_w_up, B_w_down)
    return out.reshape(B, S, D)
```
